```python
import os as _os
_os.environ.setdefault("JAX_PLATFORMS", "cpu")
import jax
import jax.numpy as jnp

def _softmax(x, axis=-1):
    return jax.nn.softmax(x, axis=axis)
def _gelu(x):
    return jax.nn.gelu(x, approximate=True)
def _silu(x):
    return jax.nn.silu(x)
def _sigmoid(x):
    return jax.nn.sigmoid(x)
def _layernorm(x, axis=-1, eps=1e-5):
    m = jnp.mean(x, axis=axis, keepdims=True)
    v = jnp.var(x, axis=axis, keepdims=True)
    return (x - m) / jnp.sqrt(v + eps)
def _scatter_add(tgt, idx, src, axis=0):
    return tgt.at[idx].add(src)
def _segment_sum(src, seg, n):
    return jax.ops.segment_sum(src, seg, n)
class _Rng:
    def __init__(self, key):
        self._k = key
    def _next(self):
        self._k, sub = jax.random.split(self._k)
        return sub
    def normal(self, shape):
        return jax.random.normal(self._next(), shape, dtype=jnp.bfloat16)
    def randint(self, lo, hi, shape):
        return jax.random.randint(self._next(), shape, lo, hi, dtype=jnp.int32)
    def uniform(self, shape, lo=0.0, hi=1.0):
        return jax.random.uniform(self._next(), shape, jnp.bfloat16, lo, hi)
    def permutation(self, n):
        return jax.random.permutation(self._next(), n)


kernel_name = 'standalone__mha_softmax__decode'

def setup_inputs():
    _rng = _Rng(jax.random.key(int.from_bytes(__import__("os").urandom(4), "little")))
    _w = (lambda a: (lambda t: t.astype(jnp.bfloat16) if jnp.issubdtype(t.dtype, jnp.floating) else t)(jnp.asarray(a)))
    B, H, Sq, Sk, D = 1, 32, 1, 8192, 128
    return {
        "q": _w((lambda *s: _rng.normal(s) * 0.8)(B, H, Sq, D)),
        "k": _w((lambda *s: _rng.normal(s) * 0.8)(B, H, Sk, D)),
        "v": _w((lambda *s: _rng.normal(s) * 0.05)(B, H, Sk, D)),
    }

def reference(q, k, v):
    scale = q.shape[-1] ** -0.5
    scores = jnp.einsum("bhqd,bhkd->bhqk", q, k) * scale
    p = _softmax(scores, axis=-1)
    return jnp.einsum("bhqk,bhkd->bhqd", p, v)
```

```python
import jax
import jax.numpy as jnp
from jax import lax
import jax.experimental.pallas as pl
import jax.experimental.pallas.tpu as pltpu

HEADS_PER_GROUP = 16
HEADS_PER_COPY = 2
ROWS_PER_COPY = 64
COPIES_PER_CHUNK = 2
LOOKAHEAD = 4


@jax.jit
def pallas_standalone__mha_softmax__decode_kernel(
    q: jax.Array,
    k: jax.Array,
    v: jax.Array,
):
    B, H, SQ, D = q.shape
    SK = k.shape[2]
    assert SQ == 1
    scale = D ** -0.5
    A, a, r, c, lag = HEADS_PER_GROUP, HEADS_PER_COPY, ROWS_PER_COPY, COPIES_PER_CHUNK, LOOKAHEAD
    G = B * H // A
    T = c * r
    cpg = SK // T
    nch = G * cpg
    nb = lag + 1

    def kernel_function(q_hbm, k_hbm, v_hbm, o_hbm, qbuf, kbuf, vbuf, obuf, ksem, vsem, qsem):
        def issue(ch):
            g, j, slot = ch // cpg, ch % cpg, ch % nb
            for i in range(c):
                off = pl.multiple_of(j * T + i * r, r)
                for b in range(A // a):
                    hs = pl.ds(b * a, a)
                    pltpu.make_async_copy(
                        v_hbm.at[g, hs, pl.ds(off, r)], vbuf.at[slot, hs, pl.ds(i * r, r)], vsem.at[slot]
                    ).start(priority=1)
                    pltpu.make_async_copy(
                        k_hbm.at[g, hs, pl.ds(off, r)], kbuf.at[slot, hs, pl.ds(i * r, r)], ksem.at[slot]
                    ).start(priority=0)

        qcopy = pltpu.make_async_copy(q_hbm, qbuf, qsem)
        qcopy.start()

        def prologue(i, carry):
            issue(i)
            return carry

        lax.fori_loop(0, lag, prologue, 0)
        qcopy.wait()

        def body(ch, carry):
            m, l, acc = carry
            g, j, slot = ch // cpg, ch % cpg, ch % nb

            @pl.when(ch + lag < nch)
            def _():
                issue(ch + lag)

            first = j == 0
            m = jnp.where(first, -jnp.inf, m)
            l = jnp.where(first, 0.0, l)
            acc = jnp.where(first, 0.0, acc)
            qg = qbuf[g]
            pltpu.make_async_copy(kbuf.at[slot], kbuf.at[slot], ksem.at[slot]).wait()
            row = lax.broadcasted_iota(jnp.int32, (A, T), 0)
            s = None
            for h in range(A):
                sh = lax.dot_general(qg, kbuf[slot, h], (((1,), (1,)), ((), ())),
                                     preferred_element_type=jnp.float32)
                s = sh if s is None else jnp.where(row == h, sh, s)
            s = s * scale
            m_new = jnp.maximum(m, jnp.max(s, axis=-1, keepdims=True))
            alpha = jnp.exp(m - m_new)
            p = jnp.exp(s - m_new)
            l = alpha * l + jnp.sum(p, axis=-1, keepdims=True)
            pb = p.astype(vbuf.dtype)
            pltpu.make_async_copy(vbuf.at[slot], vbuf.at[slot], vsem.at[slot]).wait()
            rowd = lax.broadcasted_iota(jnp.int32, (A, D), 0)
            o = None
            for h in range(A):
                oh = jnp.dot(pb, vbuf[slot, h], preferred_element_type=jnp.float32)
                o = oh if o is None else jnp.where(rowd == h, oh, o)
            acc = alpha * acc + o

            @pl.when(j == cpg - 1)
            def _():
                obuf[g] = (acc / l).astype(obuf.dtype)

            return m_new, l, acc

        init = (jnp.zeros((A, 1), jnp.float32), jnp.zeros((A, 1), jnp.float32), jnp.zeros((A, D), jnp.float32))
        lax.fori_loop(0, nch, body, init)
        ocopy = pltpu.make_async_copy(obuf, o_hbm, qsem)
        ocopy.start()
        ocopy.wait()

    out = pl.pallas_call(
        kernel_function,
        in_specs=[pl.BlockSpec(memory_space=pltpu.HBM)] * 3,
        out_specs=pl.BlockSpec(memory_space=pltpu.HBM),
        out_shape=jax.ShapeDtypeStruct((G, A, D), q.dtype),
        scratch_shapes=[
            pltpu.VMEM((G, A, D), q.dtype),
            pltpu.VMEM((nb, A, T, D), k.dtype),
            pltpu.VMEM((nb, A, T, D), v.dtype),
            pltpu.VMEM((G, A, D), q.dtype),
            pltpu.SemaphoreType.DMA((nb,)),
            pltpu.SemaphoreType.DMA((nb,)),
            pltpu.SemaphoreType.DMA(()),
        ],
        compiler_params=pltpu.CompilerParams(
            vmem_limit_bytes=2 * nb * A * T * D * 2 + 8 * 2**20,
            disable_bounds_checks=True,
            disable_semaphore_checks=True,
        ),
    )(q.reshape(G, A, D), k.reshape(G, A, SK, D), v.reshape(G, A, SK, D))
    return out.reshape(q.shape)
```

```python
import jax
import jax.numpy as jnp
from jax import lax
import jax.experimental.pallas as pl
import jax.experimental.pallas.tpu as pltpu

GROUP = 8
ROWS = 64
TILE = 2 * ROWS
SWEEPS = 2
LOOKAHEAD = 3
PRIORITIES = (1, 1, 1, 0)
QUEUE_DEPTH = 25
FIRST_HEAD = 1
TAIL_MXU, TAIL_VPU = 4, (2, 1, 1)


def _enqueue_order(num_chunks):
    regular = [(h, w, half) for w in range(SWEEPS) for h in range(GROUP) for half in range(2)]
    by_head = [(h, w, half) for h in range(GROUP) for half in range(2) for w in range(SWEEPS)]
    copies = [
        (chunk, *piece, PRIORITIES[i % len(PRIORITIES)])
        for chunk in range(num_chunks - 1)
        for i, piece in enumerate(regular)
    ]
    copies += [(num_chunks - 1, *piece, 1) for piece in by_head]
    queued = [copy for copy in copies if copy[-1] == 1]
    steps = [[] for _ in range(num_chunks)]
    taken = QUEUE_DEPTH
    for copy in copies:
        if copy[-1] == 0:
            steps[copy[0]].append(copy)
        elif taken < len(queued):
            steps[copy[0]].append(queued[taken])
            taken += 1
    return queued[:QUEUE_DEPTH], steps


@jax.jit
def pallas_standalone__mha_softmax__decode_kernel(
    q: jax.Array,
    k: jax.Array,
    v: jax.Array,
):
    batch, heads, q_len, dim = q.shape
    kv_len = k.shape[2]
    heads = batch * heads
    assert q_len == 1 and dim == TILE and heads % GROUP == 0 and kv_len % (SWEEPS * TILE) == 0
    scale = dim**-0.5
    groups = heads // GROUP
    per_group = kv_len // (SWEEPS * TILE)
    n = groups * per_group
    first, steps = _enqueue_order(2 * n)
    span = max(copy[0] for copy in steps[0])
    slots = LOOKAHEAD + span + 1
    tail = [range(TAIL_MXU)]
    for count in TAIL_VPU:
        tail.append(range(tail[-1].stop, tail[-1].stop + count))
    assert tail[-1].stop == GROUP and n > slots

    def kernel_function(
        q_hbm, k_hbm, v_hbm, o_hbm, io_ref, kv_ref, s_ref, p_ref, pt_ref, row_ref, sems, tail_sems, io_sem
    ):
        def split(c):
            if isinstance(c, int):
                return divmod(c, per_group)
            return lax.div(c, per_group), lax.rem(c, per_group)

        def start(src_hbm, c, slot, h, w, half, priority, sem):
            g, j = split(c)
            head = g * GROUP + (h + FIRST_HEAD)
            if h + FIRST_HEAD >= GROUP:
                head = head % heads if isinstance(head, int) else lax.rem(head, heads)
            pltpu.make_async_copy(
                src_hbm.at[head, half, j, w], kv_ref.at[slot, h, w, pl.ds(half * ROWS, ROWS)], sem
            ).start(priority=priority)

        def enqueue_static(copies):
            for chunk, h, w, half, priority in copies:
                if chunk == 2 * n - 1:
                    sem = tail_sems.at[[h in part for part in tail].index(True)]
                else:
                    sem = sems.at[chunk % slots]
                start((k_hbm, v_hbm)[chunk // n], chunk % n, chunk % slots, h, w, half, priority, sem)

        def enqueue(src_hbm, c, step):
            slot = [lax.rem(step + d, slots) for d in range(span + 1)]
            for d, h, w, half, priority in steps[0]:
                start(src_hbm, c + d, slot[d], h, w, half, priority, sems.at[slot[d]])

        def enqueue_at(step, lo, hi):
            for i in range(lo, hi):
                if steps[i]:
                    pl.when(step == i)(lambda i=i: enqueue_static(steps[i]))

        def wait(dst_ref, sem):
            pltpu.make_async_copy(dst_ref, dst_ref, sem).wait()

        enqueue_static(first)
        q_copy = pltpu.make_async_copy(q_hbm, io_ref, io_sem)
        q_copy.start()

        @pl.loop(0, LOOKAHEAD)
        def _(step):
            enqueue(k_hbm, step, step)

        q_copy.wait()
        queries = io_ref[...].astype(jnp.float32)
        if FIRST_HEAD:
            queries = jnp.concatenate([queries[FIRST_HEAD:], queries[:FIRST_HEAD]], axis=0)
        for g in range(groups):
            row_ref[g] = queries[g * GROUP : (g + 1) * GROUP]
        row = lax.broadcasted_iota(jnp.int32, (GROUP, TILE), 0)

        @pl.loop(0, n)
        def _(c):
            step = c + LOOKAHEAD
            pl.when(step < n - span)(lambda: enqueue(k_hbm, step, step))
            enqueue_at(step, n - span, n)
            pl.when(step >= n)(lambda: enqueue(v_hbm, step - n, step))

            slot = lax.rem(c, slots)
            g, j = split(c)
            wait(kv_ref.at[slot], sems.at[slot])
            queries = row_ref[g].astype(kv_ref.dtype)
            for w in range(SWEEPS):
                scores = jnp.zeros((GROUP, TILE), jnp.float32)
                for h in range(GROUP):
                    product = lax.dot_general(
                        queries,
                        kv_ref[slot, h, w],
                        (((1,), (1,)), ((), ())),
                        preferred_element_type=jnp.float32,
                    )
                    scores = jnp.where(row == h, product, scores)
                s_ref[j * SWEEPS + w] = scores * scale

            @pl.when(j == per_group - 1)
            def _():
                s = s_ref[...]
                e = jnp.exp(s - jnp.max(jnp.max(s, axis=0), axis=-1, keepdims=True))
                p_ref[g] = e * (1.0 / jnp.sum(jnp.sum(e, axis=0), axis=-1, keepdims=True))

        for h in range(TAIL_MXU, GROUP):
            for w in range(SWEEPS):
                p = p_ref[groups - 1, (per_group - 1) * SWEEPS + w, h : h + 1, :]
                pt_ref[h - TAIL_MXU, w] = jnp.broadcast_to(p, (dim, TILE)).T

        def weighted_values(g, j, slot, part, acc):
            for w in range(SWEEPS):
                p = p_ref[g, j * SWEEPS + w].astype(kv_ref.dtype)
                update = jnp.zeros_like(acc)
                for h in part:
                    product = jnp.dot(p, kv_ref[slot, h, w], preferred_element_type=jnp.float32)
                    update = jnp.where(row == h, product, update)
                acc = acc + update
            return acc

        def values_step(c, acc):
            step = n + c + LOOKAHEAD
            pl.when(step < 2 * n - span - 1)(lambda: enqueue(v_hbm, step - n, step))
            enqueue_at(step, 2 * n - span - 1, 2 * n)

            slot = lax.rem(n + c, slots)
            g, j = split(c)
            wait(kv_ref.at[slot], sems.at[slot])
            acc = weighted_values(g, j, slot, range(GROUP), jnp.where(j == 0, 0.0, acc))
            row_ref[g] = acc
            return acc

        acc = lax.fori_loop(0, n - 1, values_step, jnp.zeros((GROUP, dim), jnp.float32))

        finished = [row_ref[g] for g in range(groups - 1)]
        slot = (2 * n - 1) % slots
        for i, part in enumerate(tail):
            wait(kv_ref.at[slot, pl.ds(part.start, len(part))], tail_sems.at[i])
            if i == 0:
                acc = weighted_values(groups - 1, per_group - 1, slot, part, acc)
                continue
            for h in part:
                terms = []
                for w in range(SWEEPS):
                    x = kv_ref[slot, h, w].astype(jnp.float32) * pt_ref[h - TAIL_MXU, w]
                    terms += [x[r : r + 8] for r in range(0, TILE, 8)]
                while len(terms) > 1:
                    terms = [a + b for a, b in zip(terms[0::2], terms[1::2])]
                acc = jnp.where(row == h, acc + jnp.sum(terms[0], axis=0, keepdims=True), acc)

        out = jnp.concatenate(finished + [acc], axis=0)
        if FIRST_HEAD:
            out = jnp.concatenate([out[heads - FIRST_HEAD :], out[: heads - FIRST_HEAD]], axis=0)
        io_ref[...] = out.astype(io_ref.dtype)
        o_copy = pltpu.make_async_copy(io_ref, o_hbm, io_sem)
        o_copy.start()
        o_copy.wait()

    kv_shape = (heads, 2, per_group, SWEEPS, ROWS, dim)
    out = pl.pallas_call(
        kernel_function,
        in_specs=[pl.BlockSpec(memory_space=pltpu.HBM)] * 3,
        out_specs=pl.BlockSpec(memory_space=pltpu.HBM),
        out_shape=jax.ShapeDtypeStruct((heads, dim), q.dtype),
        scratch_shapes=[
            pltpu.VMEM((heads, dim), q.dtype),
            pltpu.VMEM((slots, GROUP, SWEEPS, TILE, dim), k.dtype),
            pltpu.VMEM((per_group * SWEEPS, GROUP, TILE), jnp.float32),
            pltpu.VMEM((groups, per_group * SWEEPS, GROUP, TILE), jnp.float32),
            pltpu.VMEM((GROUP - TAIL_MXU, SWEEPS, TILE, dim), jnp.float32),
            pltpu.VMEM((groups, GROUP, dim), jnp.float32),
            pltpu.SemaphoreType.DMA((slots,)),
            pltpu.SemaphoreType.DMA((len(tail),)),
            pltpu.SemaphoreType.DMA(()),
        ],
        compiler_params=pltpu.CompilerParams(disable_bounds_checks=True, disable_semaphore_checks=True),
    )(q.reshape(heads, dim), k.reshape(kv_shape), v.reshape(kv_shape))
    return out.reshape(q.shape)
```
